```python
import os as _os
_os.environ.setdefault("JAX_PLATFORMS", "cpu")
import jax
import jax.numpy as jnp

def _softmax(x, axis=-1):
    return jax.nn.softmax(x, axis=axis)
def _gelu(x):
    return jax.nn.gelu(x, approximate=True)
def _silu(x):
    return jax.nn.silu(x)
def _sigmoid(x):
    return jax.nn.sigmoid(x)
def _layernorm(x, axis=-1, eps=1e-5):
    m = jnp.mean(x, axis=axis, keepdims=True)
    v = jnp.var(x, axis=axis, keepdims=True)
    return (x - m) / jnp.sqrt(v + eps)
def _scatter_add(tgt, idx, src, axis=0):
    return tgt.at[idx].add(src)
def _segment_sum(src, seg, n):
    return jax.ops.segment_sum(src, seg, n)
class _Rng:
    def __init__(self, key):
        self._k = key
    def _next(self):
        self._k, sub = jax.random.split(self._k)
        return sub
    def normal(self, shape):
        return jax.random.normal(self._next(), shape, dtype=jnp.bfloat16)
    def randint(self, lo, hi, shape):
        return jax.random.randint(self._next(), shape, lo, hi, dtype=jnp.int32)
    def uniform(self, shape, lo=0.0, hi=1.0):
        return jax.random.uniform(self._next(), shape, jnp.bfloat16, lo, hi)
    def permutation(self, n):
        return jax.random.permutation(self._next(), n)


kernel_name = 'gated_mix__mha_block__softmax_full_mha__prompt'

def setup_inputs():
    _rng = _Rng(jax.random.key(int.from_bytes(__import__("os").urandom(4), "little")))
    _w = (lambda a: (lambda t: t.astype(jnp.bfloat16) if jnp.issubdtype(t.dtype, jnp.floating) else t)(jnp.asarray(a)))
    def _A_setup():
        B, S, D, H = 1, 2048, 448, 16
        return {
            "x": _w((lambda *s: _rng.normal(s) * 0.05)(B, S, D)),
            "wqkv": _w((lambda *s: _rng.normal(s) * 0.4)(D, 3 * D)),
            "wo": _w((lambda *s: _rng.normal(s) * 0.05)(D, D)),
        }
    _A_in = _A_setup()

    def _B_setup():
        B, S, D = 1, 2048, 448
        return {
            "x": _w((lambda *s: _rng.normal(s) * 0.05)(B, S, D)),
            "wqkv": _w((lambda *s: _rng.normal(s) * 0.4)(D, 3 * D)),
            "wo": _w((lambda *s: _rng.normal(s) * 0.05)(D, D)),
        }
    _B_in = _B_setup()

    return {
        "A_x": _A_in["x"],
        "A_wqkv": _A_in["wqkv"],
        "A_wo": _A_in["wo"],
        "B_x": _B_in["x"],
        "B_wqkv": _B_in["wqkv"],
        "B_wo": _B_in["wo"],
        "gate_w": _w((lambda *s: _rng.normal(s) * 0.05)(448) * 16.0),
    }

def reference(A_x, A_wqkv, A_wo, B_x, B_wqkv, B_wo, gate_w):
    def _A_ref(x, wqkv, wo):
        B, S, D = x.shape
        H = 16
        Dh = D // H
        qkv = (lambda x, *d: x.transpose(*d))((x @ wqkv).reshape(B, S, 3, H, Dh), 2, 0, 3, 1, 4)
        q, k, v = qkv[0], qkv[1], qkv[2]
        scores = jnp.einsum("bhqd,bhkd->bhqk", q, k) * (Dh ** -0.5)
        p = _softmax(scores, axis=-1)
        o = jnp.einsum("bhqk,bhkd->bhqd", p, v)
        return (lambda x, *d: x.transpose(*d))(o, 0, 2, 1, 3).reshape(B, S, D) @ wo

    def _B_ref(x, wqkv, wo):
        B, S, D = x.shape
        H = 16; Dh = D // H
        qkv = (lambda x, *d: x.transpose(*d))((x @ wqkv).reshape(B, S, 3, H, Dh), 2, 0, 3, 1, 4)
        q, k, v = qkv[0], qkv[1], qkv[2]
        scale = Dh ** -0.5
        scores = jnp.einsum("bhqd,bhkd->bhqk", q, k) * scale
        p = _softmax(scores, axis=-1)
        o = jnp.einsum("bhqk,bhkd->bhqd", p, v)
        return (lambda x, *d: x.transpose(*d))(o, 0, 2, 1, 3).reshape(B, S, D) @ wo

    x = A_x
    g = _sigmoid((x * gate_w).sum(-1, keepdims=True))
    a = _A_ref(x, A_wqkv, A_wo)
    b = _B_ref(x, B_wqkv, B_wo)
    return g * a + (1 - g) * b
```

```python
import functools
import math

import jax
import jax.numpy as jnp
import jax.experimental.pallas as pl
import jax.experimental.pallas.tpu as pltpu

S = 2048
D = 448
H = 16
DH = 28
DHP = 32
NH = 2 * H
NG = NH // 4
MQ = 256
NQ = S // MQ
T = NQ * NH
GROWS = 16

_F32 = jnp.float32
_BF16 = jnp.bfloat16
_QSCALE = (DH ** -0.5) * math.log2(math.e)


def _kernel(x_ref, wqv_ref, wk_ref, wo_ref, o_ref,
            k_scr, qt_scr, vt_scr, g_scr, ot_scr,
            s0, s1, m0, m1, p0, p1):
    PB = 512
    for rb in range(S // PB):
        xb = x_ref[rb * PB:(rb + 1) * PB, :]
        kb = jnp.dot(xb, wk_ref[...], preferred_element_type=_F32)
        for g in range(NG):
            k_scr[g, rb * PB:(rb + 1) * PB, :] = kb[:, g * 128:(g + 1) * 128].astype(_BF16)

    ones_rows = (jax.lax.broadcasted_iota(jnp.int32, (NH * DHP, MQ), 0) % DHP) == DH
    for qb in range(NQ):
        xb = x_ref[qb * MQ:(qb + 1) * MQ, :]
        r = jax.lax.dot_general(wqv_ref[...], xb, (((1,), (1,)), ((), ())),
                                preferred_element_type=_F32)
        qt = (r[:NH * DHP] * _QSCALE).astype(_BF16)
        for g in range(NG):
            qt_scr[qb, g] = qt[g * 128:(g + 1) * 128]
        vt = jnp.where(ones_rows, 1.0, r[NH * DHP:2 * NH * DHP])
        vt_scr[:, qb * MQ:(qb + 1) * MQ] = vt.astype(_BF16)
        g_scr[:, qb * MQ:(qb + 1) * MQ] = r[2 * NH * DHP:2 * NH * DHP + 8]

    row_grp = jax.lax.broadcasted_iota(jnp.int32, (128, MQ), 0) // DHP

    def stage_a(t, s_ref, m_ref):
        qb = t // NH
        h = t % NH
        g = h // 4
        j = h % 4
        qm = jnp.where(row_grp == j, qt_scr[qb, g], jnp.zeros((), _BF16))
        s = jnp.dot(k_scr[g], qm, preferred_element_type=_F32)
        s_ref[...] = s
        m_ref[...] = jnp.max(s, axis=0, keepdims=True)

    def stage_b(s_ref, m_ref, p_ref):
        p_ref[...] = jnp.exp2(s_ref[...] - m_ref[...]).astype(_BF16)

    def stage_c(t, p_ref):
        qb = t // NH
        h = t % NH
        r0 = pl.multiple_of(h * DHP, DHP)
        acc = jnp.dot(vt_scr[pl.ds(r0, DHP), :], p_ref[...],
                      preferred_element_type=_F32)
        l = acc[DH:DH + 1, :]
        ot_scr[qb, pl.ds(r0, DHP), :] = (acc / l).astype(_BF16)

    stage_a(0, s0, m0)
    stage_a(1, s1, m1)
    stage_b(s0, m0, p0)

    def body(u, carry):
        t = 2 * u + 1
        stage_a(t + 1, s0, m0)
        stage_b(s1, m1, p1)
        stage_c(t - 1, p0)
        stage_a(t + 2, s1, m1)
        stage_b(s0, m0, p0)
        stage_c(t, p1)
        return carry

    jax.lax.fori_loop(0, (T - 2) // 2, body, 0)
    stage_b(s1, m1, p1)
    stage_c(T - 2, p0)
    stage_c(T - 1, p1)

    for qb in range(NQ):
        ot = ot_scr[qb]
        a = jnp.dot(wo_ref[:, :H * DHP], ot[:H * DHP], preferred_element_type=_F32)
        b = jnp.dot(wo_ref[:, H * DHP:], ot[H * DHP:], preferred_element_type=_F32)
        gl = g_scr[0:1, qb * MQ:(qb + 1) * MQ]
        gate = 1.0 / (1.0 + jnp.exp(-gl))
        outT = gate * a + (1.0 - gate) * b
        o_ref[qb * MQ:(qb + 1) * MQ, :] = outT.T.astype(o_ref.dtype)


def _pad_heads(w):
    w = w.reshape(D, 3, H, DH)
    return jnp.pad(w, ((0, 0), (0, 0), (0, 0), (0, DHP - DH)))


@jax.jit
def pallas_gated_mix__mha_block__softmax_full_mha__prompt_kernel(
    A_x: jax.Array,
    A_wqkv: jax.Array,
    A_wo: jax.Array,
    B_x: jax.Array,
    B_wqkv: jax.Array,
    B_wo: jax.Array,
    gate_w: jax.Array,
):
    x = A_x.reshape(S, D)
    wa = _pad_heads(A_wqkv)
    wb = _pad_heads(B_wqkv)
    hp = H * DHP
    wq_t = jnp.concatenate([wa[:, 0].reshape(D, hp), wb[:, 0].reshape(D, hp)], axis=1).T
    wv_t = jnp.concatenate([wa[:, 2].reshape(D, hp), wb[:, 2].reshape(D, hp)], axis=1).T
    gw = jnp.pad(gate_w.reshape(1, D), ((0, GROWS - 1), (0, 0)))
    wqv = jnp.concatenate([wq_t, wv_t, gw], axis=0)
    wk = jnp.concatenate([wa[:, 1].reshape(D, hp), wb[:, 1].reshape(D, hp)], axis=1)

    def _pad_wo(w):
        w = jnp.pad(w.reshape(H, DH, D), ((0, 0), (0, DHP - DH), (0, 0)))
        return w.reshape(hp, D).T
    wo = jnp.concatenate([_pad_wo(A_wo), _pad_wo(B_wo)], axis=1)

    out = pl.pallas_call(
        _kernel,
        out_shape=jax.ShapeDtypeStruct((S, D), A_x.dtype),
        scratch_shapes=[
            pltpu.VMEM((NG, S, 128), _BF16),
            pltpu.VMEM((NQ, NG, 128, MQ), _BF16),
            pltpu.VMEM((NH * DHP, S), _BF16),
            pltpu.VMEM((8, S), _F32),
            pltpu.VMEM((NQ, NH * DHP, MQ), _BF16),
            pltpu.VMEM((S, MQ), _F32),
            pltpu.VMEM((S, MQ), _F32),
            pltpu.VMEM((1, MQ), _F32),
            pltpu.VMEM((1, MQ), _F32),
            pltpu.VMEM((S, MQ), _BF16),
            pltpu.VMEM((S, MQ), _BF16),
        ],
        compiler_params=pltpu.CompilerParams(vmem_limit_bytes=100 * 2**20),
    )(x, wqv, wk, wo)
    return out.reshape(1, S, D)
```

```python
import functools
import math
import os

import jax
import jax.numpy as jnp
import jax.experimental.pallas as pl
import jax.experimental.pallas.tpu as pltpu

S = 2048; D = 448; H = 16; DH = 28; DHP = 32; NH = 2 * H; NG = NH // 4
MQ = int(os.environ.get("MQ", 1024))
CK = int(os.environ.get("CK", 128))
UN = int(os.environ.get("UN", 2))
NQ = S // MQ
T = NQ * NH
NC = S // CK
_F32 = jnp.float32
_BF16 = jnp.bfloat16
_QSCALE = (DH ** -0.5) * math.log2(math.e)
WROWS = 4 * D + 16
PB = int(os.environ.get("PB", 512))
PQ = int(os.environ.get("PQ", 512))
OQ = int(os.environ.get("OQ", 256))
NO = S // OQ


def _shr(v, n):
    if isinstance(v, int):
        return v >> n
    return jax.lax.shift_right_logical(v, n)


def _kernel(x_hbm, wa_hbm, wb_hbm, woa_hbm, wob_hbm, gw_hbm, o_hbm,
            x_ref, wa_ref, wb_ref, woa_ref, wob_ref, gw_ref, o_ref, in_sem, out_sem,
            wt_scr, wk_scr, wot_scr, k_scr, qt_scr, vt_scr, g_scr, ot_scr,
            s0, s1, m0, m1):
    cp_wa = pltpu.make_async_copy(wa_hbm, wa_ref, in_sem.at[0])
    cp_x = pltpu.make_async_copy(x_hbm, x_ref, in_sem.at[1])
    cp_wb = pltpu.make_async_copy(wb_hbm, wb_ref, in_sem.at[2])
    cp_gw = pltpu.make_async_copy(gw_hbm, gw_ref, in_sem.at[3])
    cp_woa = pltpu.make_async_copy(woa_hbm, woa_ref, in_sem.at[4])
    cp_wob = pltpu.make_async_copy(wob_hbm, wob_ref, in_sem.at[5])
    for cp in (cp_wa, cp_x, cp_wb, cp_gw, cp_woa, cp_wob):
        cp.start()

    ej = jax.lax.broadcasted_iota(jnp.int32, (512, 512), 0) - 64
    ec = jax.lax.broadcasted_iota(jnp.int32, (512, 512), 1)
    esel = ((ec % DHP) < DH) & (ej == (ec // DHP) * DH + ec % DHP)
    e_k = jnp.where(esel, 1.0, 0.0).astype(_BF16)

    def prep(bi, w_ref):
        wk_scr[bi] = jnp.dot(w_ref[:, 384:896], e_k, preferred_element_type=_F32).astype(_BF16)
        wq = w_ref[:, 0:512].astype(_F32).T
        wt_scr[bi * D:(bi + 1) * D, :] = wq[:D].astype(_BF16)
        wv = w_ref[:, 896:1344].astype(_F32).T
        wt_scr[(2 + bi) * D:(3 + bi) * D, :] = wv.astype(_BF16)

    def kproj(bi, first):
        for rb in range(S // PB):
            cols = slice(rb * PB, (rb + 1) * PB)
            if first:
                xb = x_ref[:, cols].astype(_F32).T.astype(_BF16)
                xr_scr_set(cols, xb)
            else:
                xb = xr_scr_get(cols)
            kb = jnp.dot(xb, wk_scr[bi], preferred_element_type=_F32)
            for g in range(4):
                k_scr[4 * bi + g, cols, :] = kb[:, g * 128:(g + 1) * 128].astype(_BF16)

    xr = {}
    def xr_scr_set(cols, v):
        xr[cols.start] = v
    def xr_scr_get(cols):
        return xr[cols.start]

    cp_wa.wait()
    prep(0, wa_ref)
    cp_x.wait()
    kproj(0, True)
    cp_wb.wait()
    prep(1, wb_ref)
    kproj(1, False)
    cp_gw.wait()
    wt_scr[4 * D:4 * D + 16, :] = jnp.broadcast_to(gw_ref[...], (16, D))

    zpad = jnp.zeros((DHP - DH, PQ), _F32)
    onepad = jnp.where(jax.lax.broadcasted_iota(jnp.int32, (DHP - DH, PQ), 0) == 0, 1.0, 0.0)
    for pb in range(S // PQ):
        cols = slice(pb * PQ, (pb + 1) * PQ)
        r = jnp.dot(wt_scr[...], x_ref[:, cols], preferred_element_type=_F32)
        for g in range(NG):
            qparts = []
            for j in range(4):
                h = 4 * g + j
                qparts += [r[h * DH:(h + 1) * DH] * _QSCALE, zpad]
            qt_scr[g, :, cols] = jnp.concatenate(qparts, axis=0).astype(_BF16)
            vparts = []
            for j in range(4):
                h = 4 * g + j
                vparts += [r[2 * D + h * DH:2 * D + (h + 1) * DH], onepad]
            vt_scr[g * 128:(g + 1) * 128, cols] = jnp.concatenate(vparts, axis=0).astype(_BF16)
        gl = r[4 * D:4 * D + 8]
        gate = 1.0 / (1.0 + jnp.exp(-gl))
        g_scr[0, :, cols] = gate
        g_scr[1, :, cols] = 1.0 - gate

    cp_woa.wait()
    cp_wob.wait()
    for bi, w_ref in enumerate((woa_ref, wob_ref)):
        wot_scr[:, bi * D:(bi + 1) * D] = w_ref[...].astype(_F32).T.astype(_BF16)

    row_grp = jax.lax.broadcasted_iota(jnp.int32, (128, MQ), 0) // DHP

    def step(ta, sa, ma, tb, sb, mb):
        if ta is not None:
            qb = _shr(ta, 5); g = _shr(ta, 2) & (NG - 1); j = ta & 3
            ca = qb * MQ if isinstance(qb, int) else pl.multiple_of(qb * MQ, MQ)
            qm = jnp.where(row_grp == j, qt_scr[g, :, pl.ds(ca, MQ)], jnp.zeros((), _BF16))
            mrun = None
        if tb is not None:
            mbv = mb[...]
            qbc = _shr(tb, 5); hc = tb & (NH - 1)
            r0 = hc * DHP if isinstance(hc, int) else pl.multiple_of(hc * DHP, DHP)
            acc = None
        for c in range(NC):
            rows = slice(c * CK, (c + 1) * CK)
            if ta is not None:
                s = jnp.dot(k_scr[g, rows, :], qm, preferred_element_type=_F32)
                sa[rows, :] = s
                mc = jnp.max(s.reshape(CK // 8, 8, MQ), axis=0)
                mrun = mc if mrun is None else jnp.maximum(mrun, mc)
            if tb is not None:
                p = jnp.exp2(sb[rows, :] - mbv).astype(_BF16)
                d = jnp.dot(vt_scr[pl.ds(r0, DHP), rows], p, preferred_element_type=_F32)
                acc = d if acc is None else acc + d
        if ta is not None:
            ma[...] = jnp.max(mrun, axis=0, keepdims=True)
        if tb is not None:
            c0 = qbc * MQ if isinstance(qbc, int) else pl.multiple_of(qbc * MQ, MQ)
            gsel = g_scr[_shr(hc, 4), 0:1, pl.ds(c0, MQ)]
            scale = gsel / acc[DH:DH + 1, :]
            ot_scr[pl.ds(r0, DHP), pl.ds(c0, MQ)] = acc * scale

    bufs = ((s0, m0), (s1, m1))
    step(0, s0, m0, None, None, None)

    def body(u, carry):
        t = UN * u
        for i in range(UN):
            step(t + i + 1, *bufs[(i + 1) % 2], t + i, *bufs[i % 2])
        return carry

    n_it = (T - 1) // UN
    jax.lax.fori_loop(0, n_it, body, 0)
    for t in range(n_it * UN, T - 1):
        step(t + 1, *bufs[(t + 1) % 2], t, *bufs[t % 2])

    def out_copy(ob):
        cols = slice(ob * OQ, (ob + 1) * OQ)
        return pltpu.make_async_copy(o_ref.at[:, cols], o_hbm.at[:, cols], out_sem.at[ob])

    def oproj(ob):
        cols = slice(ob * OQ, (ob + 1) * OQ)
        parts = [ot_scr[h * DHP:h * DHP + DH, cols] for h in range(NH)]
        ot = jnp.concatenate(parts, axis=0).astype(_BF16)
        outT = jnp.dot(wot_scr[...], ot, preferred_element_type=_F32)
        o_ref[:, cols] = outT.astype(o_ref.dtype)
        out_copy(ob).start()

    n_early = (S - MQ) // OQ
    for ob in range(n_early):
        oproj(ob)
    step(None, None, None, T - 1, *bufs[(T - 1) % 2])
    for ob in range(n_early, NO):
        oproj(ob)
    for ob in range(NO):
        out_copy(ob).wait()


@jax.jit
def pallas_gated_mix__mha_block__softmax_full_mha__prompt_kernel(A_x, A_wqkv, A_wo, B_x, B_wqkv, B_wo, gate_w):
    x = jnp.transpose(A_x, (0, 2, 1)).reshape(D, S)
    any_spec = pl.BlockSpec(memory_space=pl.ANY)
    out = pl.pallas_call(
        _kernel,
        out_shape=jax.ShapeDtypeStruct((D, S), A_x.dtype),
        in_specs=[any_spec] * 6,
        out_specs=any_spec,
        scratch_shapes=[
            pltpu.VMEM((D, S), _BF16),
            pltpu.VMEM((D, 3 * D), _BF16),
            pltpu.VMEM((D, 3 * D), _BF16),
            pltpu.VMEM((D, D), _BF16),
            pltpu.VMEM((D, D), _BF16),
            pltpu.VMEM((1, D), _BF16),
            pltpu.VMEM((D, S), _BF16),
            pltpu.SemaphoreType.DMA((6,)),
            pltpu.SemaphoreType.DMA((NO,)),
            pltpu.VMEM((WROWS, D), _BF16),
            pltpu.VMEM((2, D, 512), _BF16),
            pltpu.VMEM((D, 2 * D), _BF16),
            pltpu.VMEM((NG, S, 128), _BF16),
            pltpu.VMEM((NG, 128, S), _BF16),
            pltpu.VMEM((NH * DHP, S), _BF16),
            pltpu.VMEM((2, 8, S), _F32),
            pltpu.VMEM((NH * DHP, S), _F32),
            pltpu.VMEM((S, MQ), _F32),
            pltpu.VMEM((S, MQ), _F32),
            pltpu.VMEM((1, MQ), _F32),
            pltpu.VMEM((1, MQ), _F32),
        ],
        compiler_params=pltpu.CompilerParams(vmem_limit_bytes=100 * 2**20),
    )(x, A_wqkv, B_wqkv, A_wo, B_wo, gate_w.reshape(1, D))
    return jnp.transpose(out.reshape(1, D, S), (0, 2, 1))
```

```python
import math

import jax
import jax.numpy as jnp
import jax.experimental.pallas as pl
import jax.experimental.pallas.tpu as pltpu

S = 2048
D = 448
H = 16
DH = 28
DHP = 32
NH = 2 * H
NG = NH // 4
MQ = 1024
NW = 512
CK = 128
NQ = S // MQ
T = NQ * NH
NC = S // CK
WROWS = 3 * D + 16
PQ = 512
NXC = S // PQ
OQ = 256
NO = S // OQ

_F32 = jnp.float32
_BF16 = jnp.bfloat16
_QSCALE = (DH ** -0.5) * math.log2(math.e)


def _shr(v, n):
    if isinstance(v, int):
        return v >> n
    return jax.lax.shift_right_logical(v, n)


def _aligned(v, m):
    return v if isinstance(v, int) else pl.multiple_of(v, m)


def _kernel(x_hbm, wa_hbm, wb_hbm, woa_hbm, wob_hbm, gw_hbm, o_hbm,
            x_ref, wa_ref, wb_ref, woa_ref, wob_ref, gw_ref, o_ref, in_sem, out_sem,
            wt_scr, wot_scr, k_scr, qt_scr, vt_scr, g_scr, ot_scr,
            s0, s1, m0, m1):
    cp_wa = pltpu.make_async_copy(wa_hbm, wa_ref, in_sem.at[0])
    cp_wb = pltpu.make_async_copy(wb_hbm, wb_ref, in_sem.at[1])
    cp_gw = pltpu.make_async_copy(gw_hbm, gw_ref, in_sem.at[2])
    cp_woa = pltpu.make_async_copy(woa_hbm, woa_ref, in_sem.at[3])
    cp_wob = pltpu.make_async_copy(wob_hbm, wob_ref, in_sem.at[4])
    cp_x = [pltpu.make_async_copy(x_hbm.at[:, c * PQ:(c + 1) * PQ],
                                  x_ref.at[:, c * PQ:(c + 1) * PQ],
                                  in_sem.at[5 + c]) for c in range(NXC)]
    for cp in [cp_wa, cp_gw] + cp_x + [cp_wb, cp_woa, cp_wob]:
        cp.start()

    def prep(bi, w_ref):
        for a, b in ((0, 512), (512, 1024), (1024, 3 * D)):
            wt_scr[bi, a:b, :] = w_ref[:, a:b].astype(_F32).T.astype(_BF16)
        wt_scr[bi, 3 * D:WROWS, :] = jnp.broadcast_to(gw_ref[...], (WROWS - 3 * D, D))

    zpad = jnp.zeros((DHP - DH, PQ), _F32)
    onepad = jnp.where(
        jax.lax.broadcasted_iota(jnp.int32, (DHP - DH, PQ), 0) == 0, 1.0, 0.0)

    def proj(bi):
        for pb in range(NXC):
            cols = slice(pb * PQ, (pb + 1) * PQ)
            if bi == 0:
                cp_x[pb].wait()
            r = jnp.dot(wt_scr[bi], x_ref[:, cols], preferred_element_type=_F32)
            for gg in range(4):
                g = 4 * bi + gg
                qparts, kparts, vparts = [], [], []
                for j in range(4):
                    h = 4 * gg + j
                    qparts += [r[h * DH:(h + 1) * DH] * _QSCALE, zpad]
                    kparts += [r[D + h * DH:D + (h + 1) * DH], zpad]
                    vparts += [r[2 * D + h * DH:2 * D + (h + 1) * DH], onepad]
                qt_scr[g, :, cols] = jnp.concatenate(qparts, axis=0).astype(_BF16)
                k_scr[g, cols, :] = jnp.concatenate(kparts, axis=0).T.astype(_BF16)
                vt_scr[g * 128:(g + 1) * 128, cols] = (
                    jnp.concatenate(vparts, axis=0).astype(_BF16))
            if bi == 0:
                gate = 1.0 / (1.0 + jnp.exp(-r[3 * D:3 * D + 8]))
                g_scr[0, :, cols] = gate
                g_scr[1, :, cols] = 1.0 - gate

    cp_wa.wait()
    cp_gw.wait()
    prep(0, wa_ref)
    proj(0)
    cp_wb.wait()
    prep(1, wb_ref)
    proj(1)

    cp_woa.wait()
    cp_wob.wait()
    for bi, w_ref in enumerate((woa_ref, wob_ref)):
        wot_scr[:, bi * D:(bi + 1) * D] = w_ref[...].astype(_F32).T.astype(_BF16)

    row_grp = jax.lax.broadcasted_iota(jnp.int32, (128, MQ), 0) // DHP
    nsub = MQ // NW

    def step(ta, sa, ma, tb, sb, mb):
        if ta is not None:
            g = _shr(ta, 2) & (NG - 1)
            ca = _aligned(_shr(ta, 5) * MQ, MQ)
            qm = jnp.where(row_grp == (ta & 3), qt_scr[g, :, pl.ds(ca, MQ)],
                           jnp.zeros((), _BF16))
            mrun = [None] * nsub
        if tb is not None:
            mbv = mb[...]
            r0 = _aligned((tb & (NH - 1)) * DHP, DHP)
            acc = [None] * nsub
        for c in range(NC):
            rows = slice(c * CK, (c + 1) * CK)
            for hf in range(nsub):
                cs = slice(hf * NW, (hf + 1) * NW)
                if ta is not None:
                    s = jnp.dot(k_scr[g, rows, :], qm[:, cs], preferred_element_type=_F32)
                    sa[rows, cs] = s
                    mc = jnp.max(s.reshape(CK // 8, 8, NW), axis=0)
                    mrun[hf] = mc if mrun[hf] is None else jnp.maximum(mrun[hf], mc)
                if tb is not None:
                    p = jnp.exp2(sb[rows, cs] - mbv[:, cs]).astype(_BF16)
                    d = jnp.dot(vt_scr[pl.ds(r0, DHP), rows], p,
                                preferred_element_type=_F32)
                    acc[hf] = d if acc[hf] is None else acc[hf] + d
        if ta is not None:
            ma[...] = jnp.max(jnp.concatenate(mrun, axis=1), axis=0, keepdims=True)
        if tb is not None:
            cb = _aligned(_shr(tb, 5) * MQ, MQ)
            ot_scr[pl.ds(r0, DHP), pl.ds(cb, MQ)] = jnp.concatenate(acc, axis=1)

    bufs = ((s0, m0), (s1, m1))
    step(0, s0, m0, None, None, None)

    def body(u, carry):
        t = 2 * u
        step(t + 1, s1, m1, t, s0, m0)
        step(t + 2, s0, m0, t + 1, s1, m1)
        return carry

    n_it = (T - 1) // 2
    jax.lax.fori_loop(0, n_it, body, 0)
    for t in range(2 * n_it, T - 1):
        step(t + 1, *bufs[(t + 1) % 2], t, *bufs[t % 2])

    def out_copy(ob):
        cols = slice(ob * OQ, (ob + 1) * OQ)
        return pltpu.make_async_copy(o_ref.at[:, cols], o_hbm.at[:, cols], out_sem.at[ob])

    def oproj(ob):
        cols = slice(ob * OQ, (ob + 1) * OQ)
        parts = [ot_scr[h * DHP:h * DHP + DH, cols]
                 * (g_scr[h // H, 0:1, cols] / ot_scr[h * DHP + DH:h * DHP + DH + 1, cols])
                 for h in range(NH)]
        ot = jnp.concatenate(parts, axis=0).astype(_BF16)
        out_t = jnp.dot(wot_scr[...], ot, preferred_element_type=_F32)
        o_ref[:, cols] = out_t.astype(o_ref.dtype)
        out_copy(ob).start()

    n_early = (S - MQ) // OQ
    for ob in range(n_early):
        oproj(ob)
    step(None, None, None, T - 1, *bufs[(T - 1) % 2])
    for ob in range(n_early, NO):
        oproj(ob)
    for ob in range(NO):
        out_copy(ob).wait()


@jax.jit
def pallas_gated_mix__mha_block__softmax_full_mha__prompt_kernel(
    A_x: jax.Array,
    A_wqkv: jax.Array,
    A_wo: jax.Array,
    B_x: jax.Array,
    B_wqkv: jax.Array,
    B_wo: jax.Array,
    gate_w: jax.Array,
):
    del B_x
    x_t = jnp.transpose(A_x, (0, 2, 1)).reshape(D, S)
    any_spec = pl.BlockSpec(memory_space=pl.ANY)
    out_t = pl.pallas_call(
        _kernel,
        out_shape=jax.ShapeDtypeStruct((D, S), A_x.dtype),
        in_specs=[any_spec] * 6,
        out_specs=any_spec,
        scratch_shapes=[
            pltpu.VMEM((D, S), _BF16),
            pltpu.VMEM((D, 3 * D), _BF16),
            pltpu.VMEM((D, 3 * D), _BF16),
            pltpu.VMEM((D, D), _BF16),
            pltpu.VMEM((D, D), _BF16),
            pltpu.VMEM((1, D), _BF16),
            pltpu.VMEM((D, S), _BF16),
            pltpu.SemaphoreType.DMA((5 + NXC,)),
            pltpu.SemaphoreType.DMA((NO,)),
            pltpu.VMEM((2, WROWS, D), _BF16),
            pltpu.VMEM((D, 2 * D), _BF16),
            pltpu.VMEM((NG, S, 128), _BF16),
            pltpu.VMEM((NG, 128, S), _BF16),
            pltpu.VMEM((NH * DHP, S), _BF16),
            pltpu.VMEM((2, 8, S), _F32),
            pltpu.VMEM((NH * DHP, S), _F32),
            pltpu.VMEM((S, MQ), _F32),
            pltpu.VMEM((S, MQ), _F32),
            pltpu.VMEM((1, MQ), _F32),
            pltpu.VMEM((1, MQ), _F32),
        ],
        compiler_params=pltpu.CompilerParams(vmem_limit_bytes=100 * 2**20),
    )(x_t, A_wqkv, B_wqkv, A_wo, B_wo, gate_w.reshape(1, D))
    return jnp.transpose(out_t.reshape(1, D, S), (0, 2, 1))
```
